```python
import os as _os
_os.environ.setdefault("JAX_PLATFORMS", "cpu")
import jax
import jax.numpy as jnp

def _softmax(x, axis=-1):
    return jax.nn.softmax(x, axis=axis)
def _gelu(x):
    return jax.nn.gelu(x, approximate=True)
def _silu(x):
    return jax.nn.silu(x)
def _sigmoid(x):
    return jax.nn.sigmoid(x)
def _layernorm(x, axis=-1, eps=1e-5):
    m = jnp.mean(x, axis=axis, keepdims=True)
    v = jnp.var(x, axis=axis, keepdims=True)
    return (x - m) / jnp.sqrt(v + eps)
def _scatter_add(tgt, idx, src, axis=0):
    return tgt.at[idx].add(src)
def _segment_sum(src, seg, n):
    return jax.ops.segment_sum(src, seg, n)
class _Rng:
    def __init__(self, key):
        self._k = key
    def _next(self):
        self._k, sub = jax.random.split(self._k)
        return sub
    def normal(self, shape):
        return jax.random.normal(self._next(), shape, dtype=jnp.bfloat16)
    def randint(self, lo, hi, shape):
        return jax.random.randint(self._next(), shape, lo, hi, dtype=jnp.int32)
    def uniform(self, shape, lo=0.0, hi=1.0):
        return jax.random.uniform(self._next(), shape, jnp.bfloat16, lo, hi)
    def permutation(self, n):
        return jax.random.permutation(self._next(), n)


kernel_name = 'gated_mix__mha_block__dense_activation_mish__prompt'

def setup_inputs():
    _rng = _Rng(jax.random.key(int.from_bytes(__import__("os").urandom(4), "little")))
    _w = (lambda a: (lambda t: t.astype(jnp.bfloat16) if jnp.issubdtype(t.dtype, jnp.floating) else t)(jnp.asarray(a)))
    def _A_setup():
        B, S, D, H = 1, 2048, 640, 32
        return {
            "x": _w((lambda *s: _rng.normal(s) * 0.05)(B, S, D)),
            "wqkv": _w((lambda *s: _rng.normal(s) * 0.2)(D, 3 * D)),
            "wo": _w((lambda *s: _rng.normal(s) * 0.05)(D, D)),
        }
    _A_in = _A_setup()

    def _B_setup():
        B, S, D, F = 1, 2048, 640, 1536
        return {
            "x": _w((lambda *s: _rng.normal(s) * 0.05)(B, S, D)),
            "w1": _w((lambda *s: _rng.normal(s) * 0.8)(D, F) * (D ** -0.5)),
            "b1": _w((lambda *s: _rng.normal(s) * 0.05)(F)),
            "w2": _w((lambda *s: _rng.normal(s) * 0.05)(F, D) * (F ** -0.5)),
        }
    _B_in = _B_setup()

    return {
        "A_x": _A_in["x"],
        "A_wqkv": _A_in["wqkv"],
        "A_wo": _A_in["wo"],
        "B_x": _B_in["x"],
        "B_w1": _B_in["w1"],
        "B_b1": _B_in["b1"],
        "B_w2": _B_in["w2"],
        "gate_w": _w((lambda *s: _rng.normal(s) * 0.05)(640) * 16.0),
    }

def reference(A_x, A_wqkv, A_wo, B_x, B_w1, B_b1, B_w2, gate_w):
    def _A_ref(x, wqkv, wo):
        B, S, D = x.shape
        H = 32
        Dh = D // H
        qkv = (lambda x, *d: x.transpose(*d))((x @ wqkv).reshape(B, S, 3, H, Dh), 2, 0, 3, 1, 4)
        q, k, v = qkv[0], qkv[1], qkv[2]
        scores = jnp.einsum("bhqd,bhkd->bhqk", q, k) * (Dh ** -0.5)
        p = _softmax(scores, axis=-1)
        o = jnp.einsum("bhqk,bhkd->bhqd", p, v)
        return (lambda x, *d: x.transpose(*d))(o, 0, 2, 1, 3).reshape(B, S, D) @ wo

    def _B_ref(x, w1, b1, w2):
        h = jnp.einsum("bsd,df->bsf", x, w1) + b1
        sp = jnp.log1p(jnp.exp(-jnp.abs(h))) + jnp.where(h > 0, h, jnp.zeros_like(h))
        act = h * jnp.tanh(sp)
        return jnp.einsum("bsf,fd->bsd", act, w2)

    x = A_x
    g = _sigmoid((x * gate_w).sum(-1, keepdims=True))
    a = _A_ref(x, A_wqkv, A_wo)
    b = _B_ref(x, B_w1, B_b1, B_w2)
    return g * a + (1 - g) * b
```

```python
import math

import jax
import jax.numpy as jnp
from jax import lax
import jax.experimental.pallas as pl
import jax.experimental.pallas.tpu as pltpu

_LANES = 128
_KB = 128
_QG = 512
_T1 = 512
_T3 = 512
_NT = (((1,), (1,)), ((), ()))


def _mult(i, n):
    return i if isinstance(i, int) else pl.multiple_of(i, n)


def _mish(h):
    sp = jnp.log1p(jnp.exp(-jnp.abs(h))) + jnp.where(h > 0, h, 0.0)
    return h * jnp.tanh(sp)


def _make_kernel(S, D, H, F):
    Dh = D // H
    n_tiles = D // _LANES
    n_groups = S // _QG
    straddlers = [t for t in range(n_tiles - 1) if ((t + 1) * _LANES) % Dh]
    assert straddlers == list(range(n_tiles - 1)) and Dh % 4 == 0 and Dh + 4 <= 24
    assert Dh // 2 <= _LANES // 4
    win = 24
    q_scale = (Dh**-0.5) * math.log2(math.e)

    def kernel(x_hbm, wqkv_hbm, wo_hbm, w1_hbm, b1_hbm, w2_hbm, gw_hbm, out_hbm,
               x_vm, wqkv_vm, wo_vm, w1_vm, w2_vm, wqvt, kt, qt, vt, sc, mx, ot, out_vm, b1_vm, gw_vm,
               sem_w, sem_x, sem_o):
        n1, n3 = S // _T1, S // _T3

        def x_copy(t):
            rows = pl.ds(t * _T1, _T1)
            return pltpu.make_async_copy(x_hbm.at[rows], x_vm.at[rows], sem_x.at[t])

        def out_copy(t):
            rows = pl.ds(t * _T3, _T3)
            return pltpu.make_async_copy(out_vm.at[rows], out_hbm.at[rows], sem_o.at[t])

        def wqkv_copy(i):
            cols = pl.ds(i * D, D)
            return pltpu.make_async_copy(wqkv_hbm.at[:, cols], wqkv_vm.at[:, cols], sem_w.at[5 + i])

        late_copies = [
            pltpu.make_async_copy(src, dst, sem_w.at[i])
            for i, (src, dst) in enumerate(((wo_hbm, wo_vm), (w1_hbm, w1_vm), (w2_hbm, w2_vm),
                                            (b1_hbm, b1_vm), (gw_hbm, gw_vm)))
        ]
        wqkv_copy(1).start()
        x_copy(0).start()

        def x_start(t, carry):
            x_copy(t).start()
            return carry

        lax.fori_loop(1, n1, x_start, 0)
        wqkv_copy(0).start()
        wqkv_copy(2).start()

        ot[...] = jnp.zeros_like(ot)

        wqkv_copy(1).wait()

        lane = lax.broadcasted_iota(jnp.int32, (_T1 // 2, _LANES), 1)
        row = lax.broadcasted_iota(jnp.int32, (_LANES // 2, _T1), 0)

        def k_tile(t):
            x_copy(t).wait()
            xt = x_vm[pl.ds(_mult(t * _T1, _T1), _T1), :]
            k = jnp.dot(xt, wqkv_vm[:, pl.ds(D, D)], preferred_element_type=jnp.float32)
            ku = pltpu.bitcast(k.astype(jnp.bfloat16), jnp.uint32)
            krows = pl.ds(_mult(t * (_T1 // 2), _T1 // 2), _T1 // 2)
            ktile = [ku[:, j * _LANES:(j + 1) * _LANES] for j in range(n_tiles)]
            for j in range(n_tiles):
                kt[j, krows, :] = ktile[j]
            for j in range(n_tiles - 1):
                kt[n_tiles + j, krows, :] = jnp.where(lane < _LANES // 2, ktile[j + 1], ktile[j])

        def k_body(t, carry):
            @pl.when(t == 0)
            def _():
                for c in late_copies:
                    c.start()

            k_tile(t)
            return carry

        lax.fori_loop(0, n1 - 1, k_body, 0)
        wqkv_copy(0).wait()
        wqkv_copy(2).wait()
        k_tile(n1 - 1)
        wqvt[pl.ds(0, D), :] = wqkv_vm[:, pl.ds(0, D)].T
        wqvt[pl.ds(D, D), :] = wqkv_vm[:, pl.ds(2 * D, D)].T

        def proj_body(t, carry):
            xt = x_vm[pl.ds(pl.multiple_of(t * _T1, _T1), _T1), :]
            qv = lax.dot_general(wqvt[...], xt, _NT, preferred_element_type=jnp.float32)
            cols = pl.ds(pl.multiple_of(t * _T1, _T1), _T1)
            vt[:, cols] = qv[D:, :]
            qu = pltpu.bitcast((qv[:D, :] * q_scale).astype(jnp.bfloat16), jnp.uint32)
            half = _LANES // 2
            qtile = [qu[j * half:(j + 1) * half, :] for j in range(n_tiles)]
            for j in range(n_tiles):
                qt[j, :, cols] = qtile[j]
            for j in range(n_tiles - 1):
                qt[n_tiles + j, :, cols] = jnp.where(row < half // 2, qtile[j + 1], qtile[j])
            return carry

        lax.fori_loop(0, n1, proj_body, 0)

        qrow = lax.broadcasted_iota(jnp.int32, (_LANES // 2, _QG), 0)
        vrow = lax.broadcasted_iota(jnp.int32, (win, _KB), 0)
        orow = lax.broadcasted_iota(jnp.int32, (win, _QG), 0)

        def head_step(h_qk, h_pv):
            if h_qk is not None:
                t0 = (Dh * h_qk) // _LANES
                t1 = (Dh * h_qk + Dh - 1) // _LANES
                tile = jnp.where(t0 == t1, t0, n_tiles + t0)
                lo = (Dh // 2) * h_qk - (_LANES // 2) * t0
                qmask = ((qrow - lo) & (_LANES // 2 - 1)) < Dh // 2
            if h_pv is not None:
                off = (Dh * h_pv) % 8
                w0 = pl.multiple_of(Dh * h_pv - off, 8)
                ones_row = jnp.where(off == 0, Dh, 0)
                vsel = vrow == ones_row
            for g in range(n_groups):
                qcols = pl.ds(g * _QG, _QG)
                if h_qk is not None:
                    qm = pltpu.bitcast(
                        jnp.where(qmask, qt[tile, :, qcols], jnp.uint32(0)), jnp.bfloat16)
                    m_run = jnp.full((8, _QG), -jnp.inf, jnp.float32)
                if h_pv is not None:
                    m_cur = jnp.max(mx[:, qcols], axis=0, keepdims=True)
                    acc = jnp.zeros((win, _QG), jnp.float32)
                for j in range(S // _KB):
                    keys = pl.ds(j * _KB, _KB)
                    if h_pv is not None:
                        p = jnp.exp2(sc[g, keys, :] - m_cur)
                        lhs = jnp.where(vsel, 1.0, vt[pl.ds(w0, win), keys])
                        acc = acc + jnp.dot(lhs, p, preferred_element_type=jnp.float32)
                    if h_qk is not None:
                        kb = pltpu.bitcast(kt[tile, pl.ds(j * _KB // 2, _KB // 2), :], jnp.bfloat16)
                        s = jnp.dot(kb, qm, preferred_element_type=jnp.float32)
                        m_run = jnp.maximum(m_run, jnp.max(s.reshape(_KB // 8, 8, _QG), axis=0))
                        sc[g, keys, :] = s
                if h_pv is not None:
                    den = jnp.where(off == 0, acc[Dh:Dh + 1, :], acc[0:1, :])
                    o = acc * (1.0 / den)
                    prev = ot[pl.ds(w0, win), qcols]
                    ot[pl.ds(w0, win), qcols] = jnp.where(orow >= off, o, prev)
                if h_qk is not None:
                    mx[:, qcols] = m_run

        head_step(0, None)

        def head_body(h, carry):
            head_step(h, h - 1)
            return carry

        lax.fori_loop(1, H, head_body, 0)
        head_step(None, H - 1)

        for c in late_copies:
            c.wait()
        b1 = b1_vm[...].astype(jnp.float32).reshape(1, F)
        gw = gw_vm[...].astype(jnp.float32).reshape(1, D)

        def out_body(t, carry):
            rows = pl.ds(pl.multiple_of(t * _T3, _T3), _T3)
            xt = x_vm[rows, :]
            hid = jnp.dot(xt, w1_vm[...], preferred_element_type=jnp.float32) + b1
            o = ot[:, rows].T.astype(jnp.bfloat16)
            a = jnp.dot(o, wo_vm[...], preferred_element_type=jnp.float32)
            act = _mish(hid).astype(jnp.bfloat16)
            b = jnp.dot(act, w2_vm[...], preferred_element_type=jnp.float32)
            g = jax.nn.sigmoid(jnp.sum(xt.astype(jnp.float32) * gw, axis=-1, keepdims=True))
            out_vm[rows, :] = (g * a + (1.0 - g) * b).astype(out_vm.dtype)
            out_copy(t).start()
            return carry

        lax.fori_loop(0, n3, out_body, 0)
        for t in range(n3):
            out_copy(t).wait()

    return kernel


@jax.jit
def pallas_gated_mix__mha_block__dense_activation_mish__prompt_kernel(
    A_x: jax.Array,
    A_wqkv: jax.Array,
    A_wo: jax.Array,
    B_x: jax.Array,
    B_w1: jax.Array,
    B_b1: jax.Array,
    B_w2: jax.Array,
    gate_w: jax.Array,
):
    del B_x
    B, S, D = A_x.shape
    F = B_w1.shape[1]
    H = 32
    assert B == 1 and S % _QG == 0 and S % _T1 == 0 and S % _T3 == 0 and D % _LANES == 0
    n_tiles = D // _LANES
    hbm = pl.BlockSpec(memory_space=pl.ANY)
    bf16, f32, u32 = jnp.bfloat16, jnp.float32, jnp.uint32
    out = pl.pallas_call(
        _make_kernel(S, D, H, F),
        out_shape=jax.ShapeDtypeStruct((S, D), A_x.dtype),
        in_specs=[hbm] * 7,
        out_specs=hbm,
        scratch_shapes=[
            pltpu.VMEM((S, D), bf16),
            pltpu.VMEM((D, 3 * D), bf16),
            pltpu.VMEM((D, D), bf16),
            pltpu.VMEM((D, F), bf16),
            pltpu.VMEM((F, D), bf16),
            pltpu.VMEM((2 * D, D), bf16),
            pltpu.VMEM((2 * n_tiles - 1, S // 2, _LANES), u32),
            pltpu.VMEM((2 * n_tiles - 1, _LANES // 2, S), u32),
            pltpu.VMEM((D, S), f32),
            pltpu.VMEM((S // _QG, S, _QG), f32),
            pltpu.VMEM((8, S), f32),
            pltpu.VMEM((D, S), f32),
            pltpu.VMEM((S, D), A_x.dtype),
            pltpu.VMEM((F,), bf16),
            pltpu.VMEM((D,), bf16),
            pltpu.SemaphoreType.DMA((8,)),
            pltpu.SemaphoreType.DMA((S // _T1,)),
            pltpu.SemaphoreType.DMA((S // _T3,)),
        ],
        compiler_params=pltpu.CompilerParams(vmem_limit_bytes=100 * 1024 * 1024),
    )(A_x.reshape(S, D), A_wqkv, A_wo, B_w1, B_b1, B_w2, gate_w)
    return out.reshape(B, S, D)
```
